```python
import jax
import jax.numpy as jnp

def _softmax(x, axis=-1):
    return jax.nn.softmax(x, axis=axis)
def _gelu(x):
    return jax.nn.gelu(x, approximate=True)
def _silu(x):
    return jax.nn.silu(x)
def _sigmoid(x):
    return jax.nn.sigmoid(x)
def _layernorm(x, axis=-1, eps=1e-5):
    m = jnp.mean(x, axis=axis, keepdims=True)
    v = jnp.var(x, axis=axis, keepdims=True)
    return (x - m) / jnp.sqrt(v + eps)
def _scatter_add(tgt, idx, src, axis=0):
    return tgt.at[idx].add(src)
def _segment_sum(src, seg, n):
    return jax.ops.segment_sum(src, seg, n)
class _Rng:
    def __init__(self, key):
        self._k = key
    def _next(self):
        self._k, sub = jax.random.split(self._k)
        return sub
    def normal(self, shape):
        return jax.random.normal(self._next(), shape, dtype=jnp.bfloat16)
    def randint(self, lo, hi, shape):
        return jax.random.randint(self._next(), shape, lo, hi, dtype=jnp.int32)
    def uniform(self, shape, lo=0.0, hi=1.0):
        return jax.random.uniform(self._next(), shape, jnp.bfloat16, lo, hi)
    def permutation(self, n):
        return jax.random.permutation(self._next(), n)


kernel_name = 'concat_heads__spectral_gfnet__compressed_kv_cla__prompt'

def setup_inputs():
    _rng = _Rng(jax.random.key(int.from_bytes(__import__("os").urandom(4), "little")))
    _w = (lambda a: (lambda t: t.astype(jnp.bfloat16) if jnp.issubdtype(t.dtype, jnp.floating) else t)(jnp.asarray(a)))
    def _A_setup():
        B, S, D = 1, 2048, 448
        Df = D // 2 + 1
        return {
            "x": _w((lambda *s: _rng.normal(s) * 0.05)(B, S, D)),
            "w_r": _w((lambda *s: _rng.normal(s) * 0.05)(S, Df) * 0.02),
            "w_i": _w((lambda *s: _rng.normal(s) * 0.05)(S, Df) * 0.02),
        }
    _A_in = _A_setup()

    def _B_setup():
        B, H, Sq, Sk, D, M = 1, 16, 2048, 2048, 256, 448
        Dc = 4 * D
        return {
            "x": _w((lambda *s: _rng.normal(s) * 0.05)(B, Sq, M)),
            "c_kv": _w((lambda *s: _rng.normal(s) * 0.05)(B, Sk, Dc)),
            "w_q": _w((lambda *s: _rng.normal(s) * 0.05)(M, H, D) * (M ** -0.5)),
            "w_uk": _w((lambda *s: _rng.normal(s) * 0.05)(Dc, H, D) * (Dc ** -0.5)),
            "w_uv": _w((lambda *s: _rng.normal(s) * 0.05)(Dc, H, D) * (Dc ** -0.5)),
            "w_o": _w((lambda *s: _rng.normal(s) * 0.05)(H, D, M) * ((H * D) ** -0.5)),
        }
    _B_in = _B_setup()

    return {
        "A_x": _A_in["x"],
        "A_w_r": _A_in["w_r"],
        "A_w_i": _A_in["w_i"],
        "B_x": _B_in["x"],
        "B_c_kv": _B_in["c_kv"],
        "B_w_q": _B_in["w_q"],
        "B_w_uk": _B_in["w_uk"],
        "B_w_uv": _B_in["w_uv"],
        "B_w_o": _B_in["w_o"],
    }

def reference(A_x, A_w_r, A_w_i, B_x, B_c_kv, B_w_q, B_w_uk, B_w_uv, B_w_o):
    def _A_ref(x, w_r, w_i):
        B, S, D = x.shape
        X = (lambda x, axes=(-2,-1): jnp.fft.rfft2(x.astype(jnp.float32), axes=axes))(x, axes=(-2, -1))
        W = w_r + 1j * w_i
        X = X * W
        y = (lambda x, s, axes=(-2,-1): jnp.fft.irfft2(x, s=s, axes=axes).astype(jnp.bfloat16))(X, (S, D), axes=(-2, -1))
        return y

    def _B_ref(x, c_kv, w_q, w_uk, w_uv, w_o):
        B, Sq, M = x.shape[0], x.shape[1], x.shape[2]
        Sk = c_kv.shape[1]
        H, D = w_q.shape[1], w_q.shape[2]
        q = jnp.einsum("bqm,mhd->bhqd", x, w_q)
        k = jnp.einsum("bkc,chd->bhkd", c_kv, w_uk)
        v = jnp.einsum("bkc,chd->bhkd", c_kv, w_uv)
        scores = jnp.einsum("bhqd,bhkd->bhqk", q, k) * (D ** -0.5)
        off = Sk - Sq
        qi = jnp.arange(Sq)[:, None]
        kj = jnp.arange(Sk)[None, :]
        cmask = kj <= (qi + off)
        scores = jnp.where(cmask[None, None], scores, -1e9)
        p = _softmax(scores, axis=-1)
        ctx = jnp.einsum("bhqk,bhkd->bhqd", p, v)
        return jnp.einsum("bhqd,hdm->bqm", ctx, w_o)

    a = _A_ref(A_x, A_w_r, A_w_i)
    b = _B_ref(B_x, B_c_kv, B_w_q, B_w_uk, B_w_uv, B_w_o)
    return jnp.concatenate([a, b], axis=-1)
```

```python
import jax
import jax.numpy as jnp
import ml_dtypes
import numpy as np
from jax import lax
import jax.experimental.pallas as pl
import jax.experimental.pallas.tpu as pltpu

bf16 = jnp.bfloat16
f32 = jnp.float32
u32 = jnp.uint32

S = 2048
DM = 448
F = 225
N1, N2 = 16, 128
H, HD = 16, 256
DC = 1024
NT = (((1,), (1,)), ((), ()))
NEG = -1e30


def _dft_constants():
    d = np.arange(DM)[:, None]
    f = np.arange(F)[None, :]
    th = 2 * np.pi * ((d * f) % DM) / DM
    fd = np.zeros((DM, 512))
    fd[:, :F] = np.cos(th)
    fd[:, 256:256 + F] = -np.sin(th)
    k1 = np.arange(N1)[:, None, None]
    k2 = np.arange(N2)[None, :, None]
    n2 = np.arange(N2)[None, None, :]
    ang = 2 * np.pi * ((n2 * (k1 + N1 * k2)) % S) / S
    gr, gi_ = np.cos(ang), -np.sin(ang)
    gf = np.zeros((N1, 256, 256))
    gf[:, :128, 0::2] = gr
    gf[:, :128, 1::2] = -gi_
    gf[:, 128:, 0::2] = gi_
    gf[:, 128:, 1::2] = gr
    grt, git = gr.transpose(0, 2, 1), gi_.transpose(0, 2, 1)
    gi = np.zeros((N1, 256, 256))
    gi[:, :128, 0::2] = grt
    gi[:, :128, 1::2] = git
    gi[:, 128:, 0::2] = -git
    gi[:, 128:, 1::2] = grt
    c = np.full(F, 2.0)
    c[0] = 1
    c[-1] = 1
    gdt = np.zeros((DM, 512))
    gdt[:, :F] = c[None, :] * np.cos(th) / (S * DM)
    gdt[:, 256:256 + F] = -c[None, :] * np.sin(th) / (S * DM)
    cv = lambda a: a.astype(np.float32).astype(ml_dtypes.bfloat16)
    return cv(fd), cv(gf), cv(gi), cv(gdt)


_FD, _GF, _GI, _GDT = _dft_constants()


class _SV:
    __slots__ = ("v", "s")

    def __init__(self, v, s=1):
        self.v = v
        self.s = s

    def __neg__(self):
        return _SV(self.v, -self.s)

    def __add__(self, b):
        if self.s > 0 and b.s > 0:
            return _SV(self.v + b.v)
        if self.s > 0:
            return _SV(self.v - b.v)
        if b.s > 0:
            return _SV(b.v - self.v)
        return _SV(self.v + b.v, -1)

    def __sub__(self, b):
        return self + (-b)

    def scale(self, c):
        return _SV(self.v * np.float32(abs(c)), self.s * (1 if c > 0 else -1))

    def get(self):
        return self.v if self.s > 0 else -self.v


def _twiddle(x, j, n, sign):
    re, im = x
    j %= n
    if j == 0:
        return x
    if 4 * j == n:
        return (im, -re) if sign < 0 else (-im, re)
    if 2 * j == n:
        return (-re, -im)
    if 4 * j == 3 * n:
        return (-im, re) if sign < 0 else (im, -re)
    c = np.cos(2 * np.pi * j / n)
    s = sign * np.sin(2 * np.pi * j / n)
    if (8 * j) % n == 0:
        h = np.sqrt(0.5)
        r = (re if c > 0 else -re) - (im if s > 0 else -im)
        i = (im if c > 0 else -im) + (re if s > 0 else -re)
        return (r.scale(h), i.scale(h))
    return (re.scale(c) - im.scale(s), im.scale(c) + re.scale(s))


def _fft(xs, sign):
    n = len(xs)
    if n == 1:
        return xs
    h = n // 2
    ev = [(xs[j][0] + xs[j + h][0], xs[j][1] + xs[j + h][1]) for j in range(h)]
    od = [_twiddle((xs[j][0] - xs[j + h][0], xs[j][1] - xs[j + h][1]), j, n, sign)
          for j in range(h)]
    out = [None] * n
    out[0::2] = _fft(ev, sign)
    out[1::2] = _fft(od, sign)
    return out


def _lo(u):
    return pltpu.bitcast(u << 16, f32)


def _hi(u):
    return pltpu.bitcast(u & np.uint32(0xFFFF0000), f32)


def _spectral(xa_hbm, wr_hbm, wi_hbm, fd_hbm, gf_hbm, gi_hbm, gdt_hbm, at_ref, start_b):
    def body(xa, wraw, fd, gf, gi, gdt, x1, upk, vv, wu, sem):
        cp_fd = pltpu.make_async_copy(fd_hbm, fd, sem.at[0])
        cp_xa = [pltpu.make_async_copy(xa_hbm.at[:, pl.ds(c * 512, 512)],
                                       xa.at[:, pl.ds(c * 512, 512)], sem.at[1 + c])
                 for c in range(4)]
        cp_gf = pltpu.make_async_copy(gf_hbm, gf, sem.at[5])
        cp_wr = pltpu.make_async_copy(wr_hbm, wraw.at[0], sem.at[6])
        cp_wi = pltpu.make_async_copy(wi_hbm, wraw.at[1], sem.at[7])
        cp_gi = pltpu.make_async_copy(gi_hbm, gi, sem.at[8])
        cp_gd = pltpu.make_async_copy(gdt_hbm, gdt, sem.at[9])
        cp_fd.start()
        for c in cp_xa:
            c.start()
        cp_gf.start()
        cp_wr.start()
        cp_wi.start()
        cp_gi.start()
        cp_gd.start()
        start_b()
        cp_fd.wait()
        for c in range(4):
            cp_xa[c].wait()
            xs = xa[:, c * 512:(c + 1) * 512].T
            x1[c * 512:(c + 1) * 512, :] = jnp.dot(xs, fd[...], preferred_element_type=f32)
        for r8 in range(16):
            for t in range(2):
                rows = lambda n: slice(128 * n + 8 * r8, 128 * n + 8 * r8 + 8)
                xs = [(_SV(x1[rows(n), 128 * t:128 * t + 128]),
                       _SV(x1[rows(n), 256 + 128 * t:256 + 128 * t + 128])) for n in range(16)]
                ys = _fft(xs, -1)
                for k in range(16):
                    upk[rows(k), 128 * t:128 * t + 128] = pltpu.pack_elementwise(
                        [ys[k][0].get(), ys[k][1].get()], packed_dtype=bf16)
        cp_wr.wait()
        cp_wi.wait()
        for a in range(2):
            w = jnp.concatenate([wraw[a], jnp.zeros((256 - F, S), bf16)], axis=0).T
            w = pltpu.bitcast(w, u32)
            wu[a * 2] = w[:, :128]
            wu[a * 2 + 1] = w[:, 128:]
        cp_gf.wait()
        cp_gi.wait()
        for j in range(8):
            wq = [jnp.concatenate([wu[a * 2 + t, pl.ds(j, 128, stride=8), :] for t in range(2)],
                                  axis=1) for a in range(2)]
            for b in range(2):
                k1 = 2 * j + b
                y = jnp.dot(gf[k1], pltpu.bitcast(upk[128 * k1:128 * k1 + 128, :], bf16),
                            preferred_element_type=f32)
                yr, yi = y[:128], y[128:]
                wr, wi = [(_lo if b == 0 else _hi)(w) for w in wq]
                zr = yr * wr - yi * wi
                zi = yr * wi + yi * wr
                zp = pltpu.bitcast(pltpu.pack_elementwise([zr, zi], packed_dtype=bf16), bf16)
                v = jnp.dot(gi[k1], zp, preferred_element_type=f32)
                vv[128 * k1:128 * k1 + 128, 0:256] = v[:128]
                vv[128 * k1:128 * k1 + 128, 256:512] = v[128:]
        for r8 in range(16):
            for t in range(2):
                rows = lambda n: slice(128 * n + 8 * r8, 128 * n + 8 * r8 + 8)
                xs = [(_SV(vv[rows(n), 128 * t:128 * t + 128]),
                       _SV(vv[rows(n), 256 + 128 * t:256 + 128 * t + 128])) for n in range(16)]
                ys = _fft(xs, +1)
                for k in range(16):
                    x1[rows(k), 128 * t:128 * t + 128] = ys[k][0].get()
                    x1[rows(k), 256 + 128 * t:256 + 128 * t + 128] = ys[k][1].get()
        cp_gd.wait()
        for c in range(4):
            tt = x1[c * 512:(c + 1) * 512, :].astype(bf16)
            at_ref[:, c * 512:(c + 1) * 512] = lax.dot_general(
                gdt[...], tt, NT, preferred_element_type=f32).astype(bf16)

    pl.run_scoped(
        body,
        pltpu.VMEM((DM, S), bf16),
        pltpu.VMEM((2, F, S), bf16),
        pltpu.VMEM((DM, 512), bf16),
        pltpu.VMEM((N1, 256, 256), bf16),
        pltpu.VMEM((N1, 256, 256), bf16),
        pltpu.VMEM((DM, 512), bf16),
        pltpu.VMEM((S, 512), f32),
        pltpu.VMEM((S, 256), u32),
        pltpu.VMEM((S, 512), f32),
        pltpu.VMEM((4, S // 2, 128), u32),
        pltpu.SemaphoreType.DMA((10,)),
    )


def _project(lhs_ref, wu, out_ref, nrows, scale=None):
    def body(hp, _):
        u = jnp.concatenate([x[pl.ds(hp, nrows, stride=8), :] for x in wu], axis=1)
        for b in range(2):
            w = (_lo if b == 0 else _hi)(u).astype(bf16)
            col = pl.multiple_of(hp * 512 + b * 256, 256)
            r = jnp.dot(lhs_ref[...], w, preferred_element_type=f32)
            if scale is not None:
                r = r * np.float32(scale)
            out_ref[:, pl.ds(col, 256)] = r.astype(bf16)
        return 0
    lax.fori_loop(0, H // 2, body, 0)


def _attention(q_ref, k_ref, v_ref, s_ref):
    bq, ck = 256, 256
    nq, nt = S // bq, bq // 128

    def head(h, _):
        col = pl.ds(pl.multiple_of(h * HD, HD), HD)

        def phase_a(i):
            q0, buf = i * bq, i % 2
            q = q_ref[q0:q0 + bq, col]
            mx = None
            for k0 in range(0, q0, ck):
                s = lax.dot_general(q, k_ref[k0:k0 + ck, col], NT, preferred_element_type=f32)
                s_ref[buf, :, k0:k0 + ck] = s
                r = s[:, :128]
                for t in range(1, ck // 128):
                    r = jnp.maximum(r, s[:, t * 128:(t + 1) * 128])
                mx = r if mx is None else jnp.maximum(mx, r)
            dm = [None] * nt
            for u in range(nt):
                k0 = q0 + u * 128
                s = lax.dot_general(q[u * 128:, :], k_ref[k0:k0 + 128, col], NT,
                                    preferred_element_type=f32)
                r = lax.broadcasted_iota(jnp.int32, (128, 128), 0)
                c = lax.broadcasted_iota(jnp.int32, (128, 128), 1)
                d = jnp.where(c <= r, s[:128], NEG)
                s_ref[buf, u * 128:(u + 1) * 128, k0:k0 + 128] = d
                dm[u] = d if dm[u] is None else jnp.maximum(dm[u], d)
                if u + 1 < nt:
                    s_ref[buf, (u + 1) * 128:, k0:k0 + 128] = s[128:]
                    for t in range(u + 1, nt):
                        x = s[(t - u) * 128:(t - u + 1) * 128]
                        dm[t] = x if dm[t] is None else jnp.maximum(dm[t], x)
            dmc = jnp.concatenate(dm, axis=0)
            if mx is not None:
                dmc = jnp.maximum(dmc, mx)
            return jnp.max(dmc, axis=1, keepdims=True)

        def phase_b(i, m):
            q0, buf = i * bq, i % 2
            acc = l = None
            for k0 in range(0, q0, ck):
                p = jnp.exp2(s_ref[buf, :, k0:k0 + ck] - m)
                x = p[:, :128]
                for t in range(1, ck // 128):
                    x = x + p[:, t * 128:(t + 1) * 128]
                l = x if l is None else l + x
                o = jnp.dot(p.astype(bf16), v_ref[k0:k0 + ck, col], preferred_element_type=f32)
                acc = o if acc is None else acc + o
            accs, ls = [None] * nt, [None] * nt
            for u in range(nt):
                k0 = q0 + u * 128
                p = jnp.exp2(s_ref[buf, u * 128:, k0:k0 + 128] - m[u * 128:])
                o = jnp.dot(p.astype(bf16), v_ref[k0:k0 + 128, col], preferred_element_type=f32)
                for t in range(u, nt):
                    ot = o[(t - u) * 128:(t - u + 1) * 128]
                    lt = p[(t - u) * 128:(t - u + 1) * 128]
                    accs[t] = ot if accs[t] is None else accs[t] + ot
                    ls[t] = lt if ls[t] is None else ls[t] + lt
            for t in range(nt):
                a, lt = accs[t], ls[t]
                if acc is not None:
                    a = a + acc[t * 128:(t + 1) * 128]
                    lt = lt + l[t * 128:(t + 1) * 128]
                lt = jnp.sum(lt, axis=1, keepdims=True)
                q_ref[q0 + t * 128:q0 + (t + 1) * 128, col] = (a * (1.0 / lt)).astype(bf16)

        ms = [None] * nq
        ms[0] = phase_a(0)
        for i in range(nq):
            if i + 1 < nq:
                ms[i + 1] = phase_a(i + 1)
            phase_b(i, ms[i])
        return 0

    lax.fori_loop(0, H, head, 0)


def _kernel(xa_hbm, wr_hbm, wi_hbm, xb_hbm, ckv_hbm, wq_hbm, wuk_hbm, wuv_hbm, wot_hbm,
            fd_hbm, gf_hbm, gi_hbm, gdt_hbm, out_hbm,
            at, xbt, xb, ckv, wq0, wq1, wk0, wk1, wv0, wv1, wot, sem):
    def wcopies(w_hbm, d0, d1, s0):
        return [pltpu.make_async_copy(w_hbm.at[:, pl.ds(0, 128)], d0.bitcast(bf16), sem.at[s0]),
                pltpu.make_async_copy(w_hbm.at[:, pl.ds(128, 128)], d1.bitcast(bf16), sem.at[s0 + 1])]
    cp_xb = pltpu.make_async_copy(xb_hbm, xbt, sem.at[0])
    cp_ckv = pltpu.make_async_copy(ckv_hbm, ckv, sem.at[1])
    cp_wq = wcopies(wq_hbm, wq0, wq1, 2)
    cp_wk = wcopies(wuk_hbm, wk0, wk1, 4)
    cp_wv = wcopies(wuv_hbm, wv0, wv1, 6)
    cp_wo = pltpu.make_async_copy(wot_hbm, wot, sem.at[8])

    def start_b():
        cp_xb.start()
        for c in cp_wq:
            c.start()
        cp_ckv.start()
        for c in cp_wk + cp_wv:
            c.start()
        cp_wo.start()

    _spectral(xa_hbm, wr_hbm, wi_hbm, fd_hbm, gf_hbm, gi_hbm, gdt_hbm, at, start_b)

    def attn(q, k, v, s_ref, outv, osem):
        cp_xb.wait()
        xb[...] = xbt[...].T
        for c in cp_wq:
            c.wait()
        _project(xb, (wq0, wq1), q, DM, scale=np.log2(np.e) / 16.0)
        cp_ckv.wait()
        for c in cp_wk:
            c.wait()
        _project(ckv, (wk0, wk1), k, DC)
        for c in cp_wv:
            c.wait()
        _project(ckv, (wv0, wv1), v, DC)
        _attention(q, k, v, s_ref)
        cp_wo.wait()
        wo = jnp.concatenate([wot[h] for h in range(H)], axis=1)
        qc = 512
        cps = []
        for c in range(S // qc):
            rows = slice(c * qc, (c + 1) * qc)
            bt = lax.dot_general(wo, q[rows, :], NT, preferred_element_type=f32).astype(bf16)
            outv[rows, :] = jnp.concatenate([at[:, rows], bt], axis=0).T
            cp = pltpu.make_async_copy(outv.at[rows, :], out_hbm.at[rows, :], osem.at[c])
            cp.start()
            cps.append(cp)
        for cp in cps:
            cp.wait()

    pl.run_scoped(
        attn,
        pltpu.VMEM((S, H * HD), bf16),
        pltpu.VMEM((S, H * HD), bf16),
        pltpu.VMEM((S, H * HD), bf16),
        pltpu.VMEM((2, 256, S), f32),
        pltpu.VMEM((S, 2 * DM), bf16),
        pltpu.SemaphoreType.DMA((4,)),
    )


@jax.jit
def pallas_concat_heads__spectral_gfnet__compressed_kv_cla__prompt_kernel(
    A_x: jax.Array,
    A_w_r: jax.Array,
    A_w_i: jax.Array,
    B_x: jax.Array,
    B_c_kv: jax.Array,
    B_w_q: jax.Array,
    B_w_uk: jax.Array,
    B_w_uv: jax.Array,
    B_w_o: jax.Array,
):
    hbm = pl.BlockSpec(memory_space=pltpu.HBM)
    out = pl.pallas_call(
        _kernel,
        out_shape=jax.ShapeDtypeStruct((S, 2 * DM), bf16),
        in_specs=[hbm] * 13,
        out_specs=hbm,
        scratch_shapes=[
            pltpu.VMEM((DM, S), bf16),
            pltpu.VMEM((DM, S), bf16),
            pltpu.VMEM((S, DM), bf16),
            pltpu.VMEM((S, DC), bf16),
            pltpu.VMEM((DM * H // 2, 128), u32),
            pltpu.VMEM((DM * H // 2, 128), u32),
            pltpu.VMEM((DC * H // 2, 128), u32),
            pltpu.VMEM((DC * H // 2, 128), u32),
            pltpu.VMEM((DC * H // 2, 128), u32),
            pltpu.VMEM((DC * H // 2, 128), u32),
            pltpu.VMEM((H, DM, HD), bf16),
            pltpu.SemaphoreType.DMA((9,)),
        ],
        compiler_params=pltpu.CompilerParams(vmem_limit_bytes=120 * 2**20),
        name="gfnet_cla",
    )(
        A_x[0].T, A_w_r.T, A_w_i.T, B_x[0].T, B_c_kv[0],
        B_w_q.reshape(DM * H, HD), B_w_uk.reshape(DC * H, HD), B_w_uv.reshape(DC * H, HD),
        B_w_o.transpose(0, 2, 1),
        jnp.asarray(_FD), jnp.asarray(_GF), jnp.asarray(_GI), jnp.asarray(_GDT),
    )
    return out.reshape(1, S, 2 * DM)
```

```python
import contextlib

import jax
import jax.numpy as jnp
import ml_dtypes
import numpy as np
from jax import lax
import jax.experimental.pallas as pl
import jax.experimental.pallas.tpu as pltpu

bf16 = jnp.bfloat16
f32 = jnp.float32
u32 = jnp.uint32

S = 2048
DM = 448
F = 225
N1, N2 = 16, 128
H, HD = 16, 256
DC = 1024
NT = (((1,), (1,)), ((), ()))
NEG = -1e30
_SCOPES = [False]


def _scope(name):
    return jax.named_scope(name) if _SCOPES[0] else contextlib.nullcontext()


def _dft_constants():
    d = np.arange(DM)[:, None]
    f = np.arange(F)[None, :]
    th = 2 * np.pi * ((d * f) % DM) / DM
    fd = np.zeros((DM, 512))
    fd[:, :F] = np.cos(th)
    fd[:, 256:256 + F] = -np.sin(th)
    k1 = np.arange(N1)[:, None, None]
    k2 = np.arange(N2)[None, :, None]
    n2 = np.arange(N2)[None, None, :]
    ang = 2 * np.pi * ((n2 * (k1 + N1 * k2)) % S) / S
    gr, gi_ = np.cos(ang), -np.sin(ang)
    gf = np.zeros((N1, 256, 256))
    gf[:, :128, 0::2] = gr
    gf[:, :128, 1::2] = -gi_
    gf[:, 128:, 0::2] = gi_
    gf[:, 128:, 1::2] = gr
    grt, git = gr.transpose(0, 2, 1), gi_.transpose(0, 2, 1)
    gi = np.zeros((N1, 256, 256))
    gi[:, :128, 0::2] = grt
    gi[:, :128, 1::2] = git
    gi[:, 128:, 0::2] = -git
    gi[:, 128:, 1::2] = grt
    c = np.full(F, 2.0)
    c[0] = 1
    c[-1] = 1
    gdt = np.zeros((DM, 512))
    gdt[:, :F] = c[None, :] * np.cos(th) / (S * DM)
    gdt[:, 256:256 + F] = -c[None, :] * np.sin(th) / (S * DM)
    cv = lambda a: a.astype(np.float32).astype(ml_dtypes.bfloat16)
    return cv(fd), cv(gf), cv(gi), cv(gdt)


_FD, _GF, _GI, _GDT = _dft_constants()


class _SV:
    __slots__ = ("v", "s")

    def __init__(self, v, s=1):
        self.v = v
        self.s = s

    def __neg__(self):
        return _SV(self.v, -self.s)

    def __add__(self, b):
        if self.s > 0 and b.s > 0:
            return _SV(self.v + b.v)
        if self.s > 0:
            return _SV(self.v - b.v)
        if b.s > 0:
            return _SV(b.v - self.v)
        return _SV(self.v + b.v, -1)

    def __sub__(self, b):
        return self + (-b)

    def scale(self, c):
        return _SV(self.v * np.float32(abs(c)), self.s * (1 if c > 0 else -1))

    def get(self):
        return self.v if self.s > 0 else -self.v


def _twiddle(x, j, n, sign):
    re, im = x
    j %= n
    if j == 0:
        return x
    if 4 * j == n:
        return (im, -re) if sign < 0 else (-im, re)
    if 2 * j == n:
        return (-re, -im)
    if 4 * j == 3 * n:
        return (-im, re) if sign < 0 else (im, -re)
    c = np.cos(2 * np.pi * j / n)
    s = sign * np.sin(2 * np.pi * j / n)
    if (8 * j) % n == 0:
        h = np.sqrt(0.5)
        r = (re if c > 0 else -re) - (im if s > 0 else -im)
        i = (im if c > 0 else -im) + (re if s > 0 else -re)
        return (r.scale(h), i.scale(h))
    return (re.scale(c) - im.scale(s), im.scale(c) + re.scale(s))


def _fft(xs, sign):
    n = len(xs)
    if n == 1:
        return xs
    h = n // 2
    ev = [(xs[j][0] + xs[j + h][0], xs[j][1] + xs[j + h][1]) for j in range(h)]
    od = [_twiddle((xs[j][0] - xs[j + h][0], xs[j][1] - xs[j + h][1]), j, n, sign)
          for j in range(h)]
    out = [None] * n
    out[0::2] = _fft(ev, sign)
    out[1::2] = _fft(od, sign)
    return out


def _lo(u):
    return pltpu.bitcast(u << 16, f32)


def _hi(u):
    return pltpu.bitcast(u & np.uint32(0xFFFF0000), f32)


def _spectral(xa_hbm, wr_hbm, wi_hbm, fd_hbm, gf_hbm, gi_hbm, gdt_hbm, at_ref, start_b):
    def body(xa, wraw, fd, gf, gi, gdt, x1, upk, vv, wu, sem):
        cp_fd = pltpu.make_async_copy(fd_hbm, fd, sem.at[0])
        cp_xa = [pltpu.make_async_copy(xa_hbm.at[:, pl.ds(c * 512, 512)],
                                       xa.at[:, pl.ds(c * 512, 512)], sem.at[1 + c])
                 for c in range(4)]
        cp_gf = pltpu.make_async_copy(gf_hbm, gf, sem.at[5])
        cp_wr = pltpu.make_async_copy(wr_hbm, wraw.at[0], sem.at[6])
        cp_wi = pltpu.make_async_copy(wi_hbm, wraw.at[1], sem.at[7])
        cp_gi = pltpu.make_async_copy(gi_hbm, gi, sem.at[8])
        cp_gd = pltpu.make_async_copy(gdt_hbm, gdt, sem.at[9])
        cp_fd.start()
        for c in cp_xa:
            c.start()
        cp_fd.wait()
        for c in range(4):
            cp_xa[c].wait()
            if c == 0:
                for cp in (cp_wr, cp_wi, cp_gf, cp_gi, cp_gd):
                    cp.start()
            xs = xa[:, c * 512:(c + 1) * 512].T
            x1[c * 512:(c + 1) * 512, :] = jnp.dot(xs, fd[...], preferred_element_type=f32)
        for r8 in range(16):
            for t in range(2):
                rows = lambda n: slice(128 * n + 8 * r8, 128 * n + 8 * r8 + 8)
                xs = [(_SV(x1[rows(n), 128 * t:128 * t + 128]),
                       _SV(x1[rows(n), 256 + 128 * t:256 + 128 * t + 128])) for n in range(16)]
                ys = _fft(xs, -1)
                for k in range(16):
                    upk[rows(k), 128 * t:128 * t + 128] = pltpu.pack_elementwise(
                        [ys[k][0].get(), ys[k][1].get()], packed_dtype=bf16)
        cp_wr.wait()
        cp_wi.wait()
        for a in range(2):
            w = jnp.concatenate([wraw[a], jnp.zeros((256 - F, S), bf16)], axis=0).T
            w = pltpu.bitcast(w, u32)
            wu[a * 2] = w[:, :128]
            wu[a * 2 + 1] = w[:, 128:]
        cp_gf.wait()
        cp_gi.wait()
        start_b()
        for j in range(8):
            wq = [jnp.concatenate([wu[a * 2 + t, pl.ds(j, 128, stride=8), :] for t in range(2)],
                                  axis=1) for a in range(2)]
            for b in range(2):
                k1 = 2 * j + b
                y = jnp.dot(gf[k1], pltpu.bitcast(upk[128 * k1:128 * k1 + 128, :], bf16),
                            preferred_element_type=f32)
                yr, yi = y[:128], y[128:]
                wr, wi = [(_lo if b == 0 else _hi)(w) for w in wq]
                zr = yr * wr - yi * wi
                zi = yr * wi + yi * wr
                zp = pltpu.bitcast(pltpu.pack_elementwise([zr, zi], packed_dtype=bf16), bf16)
                v = jnp.dot(gi[k1], zp, preferred_element_type=f32)
                vv[128 * k1:128 * k1 + 128, 0:256] = v[:128]
                vv[128 * k1:128 * k1 + 128, 256:512] = v[128:]
        for r8 in range(16):
            for t in range(2):
                rows = lambda n: slice(128 * n + 8 * r8, 128 * n + 8 * r8 + 8)
                xs = [(_SV(vv[rows(n), 128 * t:128 * t + 128]),
                       _SV(vv[rows(n), 256 + 128 * t:256 + 128 * t + 128])) for n in range(16)]
                ys = _fft(xs, +1)
                for k in range(16):
                    x1[rows(k), 128 * t:128 * t + 128] = ys[k][0].get()
                    x1[rows(k), 256 + 128 * t:256 + 128 * t + 128] = ys[k][1].get()
        cp_gd.wait()
        for c in range(4):
            tt = x1[c * 512:(c + 1) * 512, :].astype(bf16)
            at_ref[:, c * 512:(c + 1) * 512] = lax.dot_general(
                gdt[...], tt, NT, preferred_element_type=f32).astype(bf16)

    pl.run_scoped(
        body,
        pltpu.VMEM((DM, S), bf16),
        pltpu.VMEM((2, F, S), bf16),
        pltpu.VMEM((DM, 512), bf16),
        pltpu.VMEM((N1, 256, 256), bf16),
        pltpu.VMEM((N1, 256, 256), bf16),
        pltpu.VMEM((DM, 512), bf16),
        pltpu.VMEM((S, 512), f32),
        pltpu.VMEM((S, 256), u32),
        pltpu.VMEM((S, 512), f32),
        pltpu.VMEM((4, S // 2, 128), u32),
        pltpu.SemaphoreType.DMA((10,)),
    )


def _strassen_a(get, sa_ref, rows):
    a11, a12, a21, a22 = [get(i, j, rows).astype(f32) for i in (0, 1) for j in (0, 1)]
    s1 = a21 + a22
    s2 = s1 - a11
    sa_ref[0, rows, :] = s1.astype(bf16)
    sa_ref[1, rows, :] = s2.astype(bf16)
    sa_ref[2, rows, :] = (a11 - a21).astype(bf16)
    sa_ref[3, rows, :] = (a12 - s2).astype(bf16)


def _project(get_a, sa_ref, wu, tb, out_ref, n_it, kh, k2, scale=None, extra=None):
    rc = 256
    nch = (S // 2) // rc

    def prep(it, slot, c0, cn):
        w, hp = it // 8, it % 8

        def rows(base):
            return jnp.concatenate(
                [x[w, pl.ds(hp + 8 * base, cn, stride=8), :] for x in wu], axis=1)
        ua = rows(c0)
        b11, b12 = _lo(ua), _hi(ua)
        if c0 + cn <= k2:
            ub = rows(kh + c0)
            b21, b22 = _lo(ub), _hi(ub)
            t1 = b12 - b11
            t2 = b22 - t1
            ts = [b11, b21, b22, t2 - b21, t1, t2, b22 - b12]
        else:
            assert c0 >= k2
            z = jnp.zeros_like(b11)
            t1 = b12 - b11
            ts = [b11, z, z, -t1, t1, -t1, -b12]
        for i in range(7):
            tb[slot, i, c0:c0 + cn, :] = ts[i].astype(bf16)

    def aop(i, r0):
        r = slice(r0, r0 + rc)
        return [lambda: get_a(0, 0, r), lambda: get_a(0, 1, r), lambda: sa_ref[3, r, :],
                lambda: get_a(1, 1, r), lambda: sa_ref[0, r, :], lambda: sa_ref[1, r, :],
                lambda: sa_ref[2, r, :]][i]()

    def body(it, _):
        slot = it % 2
        w, hp = it // 8, it % 8
        nxt = jnp.minimum(it + 1, n_it - 1)
        col = pl.multiple_of(hp * 512, 512)
        cn = kh // nch
        for ci in range(nch):
            r0 = ci * rc
            p1, p2, p3, p4, p5, p6, p7 = [
                jnp.dot(aop(i, r0), tb[slot, i], preferred_element_type=f32) for i in range(7)]
            u2 = p1 + p6
            u3 = u2 + p7
            res = (p1 + p2, (u2 + p5) + p3, u3 - p4, u3 + p5)
            if scale is not None:
                res = [x * np.float32(scale) for x in res]
            for n, x in enumerate(res):
                r = (n // 2) * (S // 2) + r0
                out_ref[w, r:r + rc, pl.ds(col + (n % 2) * 256, 256)] = x.astype(bf16)
            prep(nxt, 1 - slot, ci * cn, cn)
            if extra is not None:
                extra(it, ci)
        return 0

    for ci in range(nch):
        prep(0, 0, ci * (kh // nch), kh // nch)
    lax.fori_loop(0, n_it, body, 0)


def _attention(q_ref, k_ref, v_ref, s_ref):
    bq, ck = 256, 256
    nq, nt = S // bq, bq // 128

    def head(h, _):
        col = pl.ds(pl.multiple_of(h * HD, HD), HD)

        def phase_a(i):
            q0, buf = i * bq, i % 2
            q = q_ref[q0:q0 + bq, col]
            mx = None
            for k0 in range(0, q0, ck):
                s = lax.dot_general(q, k_ref[k0:k0 + ck, col], NT, preferred_element_type=f32)
                s_ref[buf, :, k0:k0 + ck] = s
                r = s[:, :128]
                for t in range(1, ck // 128):
                    r = jnp.maximum(r, s[:, t * 128:(t + 1) * 128])
                mx = r if mx is None else jnp.maximum(mx, r)
            dm = [None] * nt
            for u in range(nt):
                k0 = q0 + u * 128
                s = lax.dot_general(q[u * 128:, :], k_ref[k0:k0 + 128, col], NT,
                                    preferred_element_type=f32)
                r = lax.broadcasted_iota(jnp.int32, (128, 128), 0)
                c = lax.broadcasted_iota(jnp.int32, (128, 128), 1)
                d = jnp.where(c <= r, s[:128], NEG)
                s_ref[buf, u * 128:(u + 1) * 128, k0:k0 + 128] = d
                dm[u] = d if dm[u] is None else jnp.maximum(dm[u], d)
                if u + 1 < nt:
                    s_ref[buf, (u + 1) * 128:, k0:k0 + 128] = s[128:]
                    for t in range(u + 1, nt):
                        x = s[(t - u) * 128:(t - u + 1) * 128]
                        dm[t] = x if dm[t] is None else jnp.maximum(dm[t], x)
            dmc = jnp.concatenate(dm, axis=0)
            if mx is not None:
                dmc = jnp.maximum(dmc, mx)
            return jnp.max(dmc, axis=1, keepdims=True)

        def phase_b(i, m):
            q0, buf = i * bq, i % 2
            acc = l = None
            for k0 in range(0, q0, ck):
                p = jnp.exp2(s_ref[buf, :, k0:k0 + ck] - m)
                x = p[:, :128]
                for t in range(1, ck // 128):
                    x = x + p[:, t * 128:(t + 1) * 128]
                l = x if l is None else l + x
                o = jnp.dot(p.astype(bf16), v_ref[k0:k0 + ck, col], preferred_element_type=f32)
                acc = o if acc is None else acc + o
            accs, ls = [None] * nt, [None] * nt
            for u in range(nt):
                k0 = q0 + u * 128
                p = jnp.exp2(s_ref[buf, u * 128:, k0:k0 + 128] - m[u * 128:])
                o = jnp.dot(p.astype(bf16), v_ref[k0:k0 + 128, col], preferred_element_type=f32)
                for t in range(u, nt):
                    ot = o[(t - u) * 128:(t - u + 1) * 128]
                    lt = p[(t - u) * 128:(t - u + 1) * 128]
                    accs[t] = ot if accs[t] is None else accs[t] + ot
                    ls[t] = lt if ls[t] is None else ls[t] + lt
            for t in range(nt):
                a, lt = accs[t], ls[t]
                if acc is not None:
                    a = a + acc[t * 128:(t + 1) * 128]
                    lt = lt + l[t * 128:(t + 1) * 128]
                lt = jnp.sum(lt, axis=1, keepdims=True)
                q_ref[q0 + t * 128:q0 + (t + 1) * 128, col] = (a * (1.0 / lt)).astype(bf16)

        ms = [None] * nq
        ms[nq - 1] = phase_a(nq - 1)
        for i in range(nq - 1, -1, -1):
            if i > 0:
                ms[i - 1] = phase_a(i - 1)
            phase_b(i, ms[i])
        return 0

    lax.fori_loop(0, H, head, 0)


def _kernel(xa_hbm, wr_hbm, wi_hbm, xb_hbm, ckv_hbm, wq_hbm, wuk_hbm, wuv_hbm, wot_hbm,
            fd_hbm, gf_hbm, gi_hbm, gdt_hbm, out_hbm,
            at, xbt, xb, ckv, wq0, wq1, wk0, wk1, wot, sem):
    def wcopies(w_hbm, d0, d1, s0):
        return [pltpu.make_async_copy(w_hbm.at[:, pl.ds(0, 128)], d0.bitcast(bf16), sem.at[s0]),
                pltpu.make_async_copy(w_hbm.at[:, pl.ds(128, 128)], d1.bitcast(bf16), sem.at[s0 + 1])]
    cp_xb = pltpu.make_async_copy(xb_hbm, xbt, sem.at[0])
    cp_ckv = pltpu.make_async_copy(ckv_hbm, ckv, sem.at[1])
    cp_wq = wcopies(wq_hbm, wq0.at[0], wq1.at[0], 2)
    cp_wk = wcopies(wuk_hbm, wk0.at[0], wk1.at[0], 4)
    cp_wv = wcopies(wuv_hbm, wk0.at[1], wk1.at[1], 6)
    cp_wo = pltpu.make_async_copy(wot_hbm, wot, sem.at[8])

    def start_b():
        cp_xb.start()
        for c in cp_wq:
            c.start()
        cp_ckv.start()

    with _scope("A"):
        _spectral(xa_hbm, wr_hbm, wi_hbm, fd_hbm, gf_hbm, gi_hbm, gdt_hbm, at, start_b)

    def attn(q, kv, sx, sc, tbq, tb, s_ref, outv, osem):
        hs = S // 2
        cp_xb.wait()
        xb[:, :DM] = xbt[...].T
        xb[:, DM:] = jnp.zeros((S, 512 - DM), bf16)
        get_x = lambda i, j, r: xb[i * hs + r.start:i * hs + r.stop, j * 256:(j + 1) * 256]
        get_c = lambda i, j, r: ckv[pl.ds(i * hs + r.start, r.size), j * 512:(j + 1) * 512] \
            if not isinstance(r, slice) else ckv[i * hs + r.start:i * hs + r.stop, j * 512:(j + 1) * 512]
        _strassen_a(get_x, sx, slice(0, hs))
        for c in cp_wq:
            c.wait()
        cp_ckv.wait()
        for c in cp_wk + cp_wv:
            c.start()
        cp_wo.start()

        def extra(it, ci):
            rows = pl.ds(pl.multiple_of((it * 4 + ci) * 32, 32), 32)
            _strassen_a(get_c, sc, rows)

        with _scope("Qproj"):
            _project(get_x, sx, (wq0, wq1), tbq, q, 8, 256, 192,
                     scale=np.log2(np.e) / 16.0, extra=extra)
        for c in cp_wk + cp_wv:
            c.wait()
        with _scope("KVproj"):
            _project(get_c, sc, (wk0, wk1), tb, kv, 16, 512, 512)
        with _scope("attn"):
            _attention(q.at[0], kv.at[0], kv.at[1], s_ref)
        cp_wo.wait()
        wo = jnp.concatenate([wot[h] for h in range(H)], axis=1)
        qc = 512
        cps = []
        for c in range(S // qc):
            rows = slice(c * qc, (c + 1) * qc)
            bt = lax.dot_general(wo, q[0, rows, :], NT, preferred_element_type=f32).astype(bf16)
            outv[rows, :] = jnp.concatenate([at[:, rows], bt], axis=0).T
            cp = pltpu.make_async_copy(outv.at[rows, :], out_hbm.at[rows, :], osem.at[c])
            cp.start()
            cps.append(cp)
        for cp in cps:
            cp.wait()

    pl.run_scoped(
        attn,
        pltpu.VMEM((1, S, H * HD), bf16),
        pltpu.VMEM((2, S, H * HD), bf16),
        pltpu.VMEM((4, S // 2, 256), bf16),
        pltpu.VMEM((4, S // 2, 512), bf16),
        pltpu.VMEM((2, 7, 256, 256), bf16),
        pltpu.VMEM((2, 7, 512, 256), bf16),
        pltpu.VMEM((2, 256, S), f32),
        pltpu.VMEM((S, 2 * DM), bf16),
        pltpu.SemaphoreType.DMA((4,)),
    )


@jax.jit
def pallas_concat_heads__spectral_gfnet__compressed_kv_cla__prompt_kernel(
    A_x: jax.Array,
    A_w_r: jax.Array,
    A_w_i: jax.Array,
    B_x: jax.Array,
    B_c_kv: jax.Array,
    B_w_q: jax.Array,
    B_w_uk: jax.Array,
    B_w_uv: jax.Array,
    B_w_o: jax.Array,
):
    hbm = pl.BlockSpec(memory_space=pltpu.HBM)
    out = pl.pallas_call(
        _kernel,
        out_shape=jax.ShapeDtypeStruct((S, 2 * DM), bf16),
        in_specs=[hbm] * 13,
        out_specs=hbm,
        scratch_shapes=[
            pltpu.VMEM((DM, S), bf16),
            pltpu.VMEM((DM, S), bf16),
            pltpu.VMEM((S, 512), bf16),
            pltpu.VMEM((S, DC), bf16),
            pltpu.VMEM((1, DM * H // 2, 128), u32),
            pltpu.VMEM((1, DM * H // 2, 128), u32),
            pltpu.VMEM((2, DC * H // 2, 128), u32),
            pltpu.VMEM((2, DC * H // 2, 128), u32),
            pltpu.VMEM((H, DM, HD), bf16),
            pltpu.SemaphoreType.DMA((9,)),
        ],
        compiler_params=pltpu.CompilerParams(vmem_limit_bytes=120 * 2**20),
        name="gfnet_cla",
    )(
        A_x[0].T, A_w_r.T, A_w_i.T, B_x[0].T, B_c_kv[0],
        B_w_q.reshape(DM * H, HD), B_w_uk.reshape(DC * H, HD), B_w_uv.reshape(DC * H, HD),
        B_w_o.transpose(0, 2, 1),
        jnp.asarray(_FD), jnp.asarray(_GF), jnp.asarray(_GI), jnp.asarray(_GDT),
    )
    return out.reshape(1, S, 2 * DM)
```

```python
import contextlib
import functools

import jax
import jax.numpy as jnp
import ml_dtypes
import numpy as np
from jax import lax
import jax.experimental.pallas as pl
import jax.experimental.pallas.tpu as pltpu

bf16 = jnp.bfloat16
f32 = jnp.float32
u32 = jnp.uint32

S = 2048
DM = 448
F = 225
N1, N2 = 16, 128
H, HD = 16, 256
DC = 1024
NT = (((1,), (1,)), ((), ()))
NEG = -1e30
_SCOPES = [False]


def _scope(name):
    return jax.named_scope(name) if _SCOPES[0] else contextlib.nullcontext()


def _dft_constants():
    d = np.arange(DM)[:, None]
    f = np.arange(F)[None, :]
    th = 2 * np.pi * ((d * f) % DM) / DM
    fd = np.zeros((DM, 512))
    fd[:, :F] = np.cos(th)
    fd[:, 256:256 + F] = -np.sin(th)
    k1 = np.arange(N1)[:, None, None]
    k2 = np.arange(N2)[None, :, None]
    n2 = np.arange(N2)[None, None, :]
    ang = 2 * np.pi * ((n2 * (k1 + N1 * k2)) % S) / S
    gr, gi_ = np.cos(ang), -np.sin(ang)
    gf = np.zeros((N1, 256, 256))
    gf[:, :128, 0::2] = gr
    gf[:, :128, 1::2] = -gi_
    gf[:, 128:, 0::2] = gi_
    gf[:, 128:, 1::2] = gr
    grt, git = gr.transpose(0, 2, 1), gi_.transpose(0, 2, 1)
    gi = np.zeros((N1, 256, 256))
    gi[:, :128, 0::2] = grt
    gi[:, :128, 1::2] = git
    gi[:, 128:, 0::2] = -git
    gi[:, 128:, 1::2] = grt
    c = np.full(F, 2.0)
    c[0] = 1
    c[-1] = 1
    gdt = np.zeros((DM, 512))
    gdt[:, :F] = c[None, :] * np.cos(th) / (S * DM)
    gdt[:, 256:256 + F] = -c[None, :] * np.sin(th) / (S * DM)
    cv = lambda a: a.astype(np.float32).astype(ml_dtypes.bfloat16)
    return cv(fd), cv(gf), cv(gi), cv(gdt)


_FD, _GF, _GI, _GDT = _dft_constants()


class _SV:
    __slots__ = ("v", "s")

    def __init__(self, v, s=1):
        self.v = v
        self.s = s

    def __neg__(self):
        return _SV(self.v, -self.s)

    def __add__(self, b):
        if self.s > 0 and b.s > 0:
            return _SV(self.v + b.v)
        if self.s > 0:
            return _SV(self.v - b.v)
        if b.s > 0:
            return _SV(b.v - self.v)
        return _SV(self.v + b.v, -1)

    def __sub__(self, b):
        return self + (-b)

    def scale(self, c):
        return _SV(self.v * np.float32(abs(c)), self.s * (1 if c > 0 else -1))

    def get(self):
        return self.v if self.s > 0 else -self.v


def _twiddle(x, j, n, sign):
    re, im = x
    j %= n
    if j == 0:
        return x
    if 4 * j == n:
        return (im, -re) if sign < 0 else (-im, re)
    if 2 * j == n:
        return (-re, -im)
    if 4 * j == 3 * n:
        return (-im, re) if sign < 0 else (im, -re)
    c = np.cos(2 * np.pi * j / n)
    s = sign * np.sin(2 * np.pi * j / n)
    if (8 * j) % n == 0:
        h = np.sqrt(0.5)
        r = (re if c > 0 else -re) - (im if s > 0 else -im)
        i = (im if c > 0 else -im) + (re if s > 0 else -re)
        return (r.scale(h), i.scale(h))
    return (re.scale(c) - im.scale(s), im.scale(c) + re.scale(s))


def _fft(xs, sign):
    n = len(xs)
    if n == 1:
        return xs
    h = n // 2
    ev = [(xs[j][0] + xs[j + h][0], xs[j][1] + xs[j + h][1]) for j in range(h)]
    od = [_twiddle((xs[j][0] - xs[j + h][0], xs[j][1] - xs[j + h][1]), j, n, sign)
          for j in range(h)]
    out = [None] * n
    out[0::2] = _fft(ev, sign)
    out[1::2] = _fft(od, sign)
    return out


def _lo(u):
    return pltpu.bitcast(u << 16, f32)


def _hi(u):
    return pltpu.bitcast(u & np.uint32(0xFFFF0000), f32)


def _spectral(xa_hbm, wr_hbm, wi_hbm, fd_hbm, gf_hbm, gi_hbm, gdt_hbm, at_ref, start_b, late):
    def body(xa, wraw, fd, gf, gi, gdt, x1, upk, vv, wu, sem):
        cp_fd = pltpu.make_async_copy(fd_hbm, fd, sem.at[0])
        cp_xa = [pltpu.make_async_copy(xa_hbm.at[:, pl.ds(c * 512, 512)],
                                       xa.at[:, pl.ds(c * 512, 512)], sem.at[1 + c])
                 for c in range(4)]
        cp_wr = pltpu.make_async_copy(wr_hbm, wraw.at[0], sem.at[5])
        cp_wi = pltpu.make_async_copy(wi_hbm, wraw.at[1], sem.at[6])
        cp_gd = pltpu.make_async_copy(gdt_hbm, gdt, sem.at[7])
        cp_g = [[pltpu.make_async_copy(h.at[pl.ds(4 * j, 4)], v.at[pl.ds(4 * j, 4)],
                                       sem.at[8 + 2 * j + n])
                 for n, (h, v) in enumerate(((gf_hbm, gf), (gi_hbm, gi)))] for j in range(4)]
        cp_fd.start()
        for c in cp_xa:
            c.start()
        with _scope("A0wait"):
            cp_fd.wait()
            cp_xa[0].wait()
        for c in range(4):
            with _scope("A1_%d" % c):
                if c:
                    cp_xa[c].wait()
                if c == 0:
                    for cp in (cp_wr, cp_wi):
                        cp.start()
                if c == 1:
                    for cp in cp_g[0]:
                        cp.start()
                if c == 3:
                    for cp in cp_g[1]:
                        cp.start()
                xs = xa[:, c * 512:(c + 1) * 512].T
                x1[c * 512:(c + 1) * 512, :] = jnp.dot(xs, fd[...], preferred_element_type=f32)
        with _scope("A2"):
            for r8 in range(16):
                for t in range(2):
                    rows = lambda n: slice(128 * n + 8 * r8, 128 * n + 8 * r8 + 8)
                    xs = [(_SV(x1[rows(n), 128 * t:128 * t + 128]),
                           _SV(x1[rows(n), 256 + 128 * t:256 + 128 * t + 128])) for n in range(16)]
                    ys = _fft(xs, -1)
                    for k in range(16):
                        upk[rows(k), 128 * t:128 * t + 128] = pltpu.pack_elementwise(
                            [ys[k][0].get(), ys[k][1].get()], packed_dtype=bf16)
            cp_wr.wait()
            cp_wi.wait()
            for cp in cp_g[2]:
                cp.start()
            for a in range(2):
                w = jnp.concatenate([wraw[a], jnp.zeros((256 - F, S), bf16)], axis=0).T
                w = pltpu.bitcast(w, u32)
                wu[a * 2] = w[:, :128]
                wu[a * 2 + 1] = w[:, 128:]
        with _scope("A3"):
            for j in range(8):
                if j % 2 == 0:
                    for cp in cp_g[j // 2]:
                        cp.wait()
                if j == 0:
                    for cp in cp_g[3]:
                        cp.start()
                if j == 2:
                    cp_gd.start()
                if j == 4:
                    start_b()
                wq = [jnp.concatenate([wu[a * 2 + t, pl.ds(j, 128, stride=8), :]
                                       for t in range(2)], axis=1) for a in range(2)]
                for b in range(2):
                    k1 = 2 * j + b
                    y = jnp.dot(gf[k1], pltpu.bitcast(upk[128 * k1:128 * k1 + 128, :], bf16),
                                preferred_element_type=f32)
                    yr, yi = y[:128], y[128:]
                    wr, wi = [(_lo if b == 0 else _hi)(w) for w in wq]
                    zr = yr * wr - yi * wi
                    zi = yr * wi + yi * wr
                    zp = pltpu.bitcast(pltpu.pack_elementwise([zr, zi], packed_dtype=bf16), bf16)
                    v = jnp.dot(gi[k1], zp, preferred_element_type=f32)
                    vv[128 * k1:128 * k1 + 128, 0:256] = v[:128]
                    vv[128 * k1:128 * k1 + 128, 256:512] = v[128:]
        with _scope("A6"):
            for r8 in range(16):
                for t in range(2):
                    rows = lambda n: slice(128 * n + 8 * r8, 128 * n + 8 * r8 + 8)
                    xs = [(_SV(vv[rows(n), 128 * t:128 * t + 128]),
                           _SV(vv[rows(n), 256 + 128 * t:256 + 128 * t + 128])) for n in range(16)]
                    ys = _fft(xs, +1)
                    for k in range(16):
                        x1[rows(k), 128 * t:128 * t + 128] = ys[k][0].get()
                        x1[rows(k), 256 + 128 * t:256 + 128 * t + 128] = ys[k][1].get()
        with _scope("A7"):
            cp_gd.wait()
            for c in range(4):
                tt = x1[c * 512:(c + 1) * 512, :].astype(bf16)
                at_ref[:, c * 512:(c + 1) * 512] = lax.dot_general(
                    gdt[...], tt, NT, preferred_element_type=f32).astype(bf16)
                late(c)

    pl.run_scoped(
        body,
        pltpu.VMEM((DM, S), bf16),
        pltpu.VMEM((2, F, S), bf16),
        pltpu.VMEM((DM, 512), bf16),
        pltpu.VMEM((N1, 256, 256), bf16),
        pltpu.VMEM((N1, 256, 256), bf16),
        pltpu.VMEM((DM, 512), bf16),
        pltpu.VMEM((S, 512), f32),
        pltpu.VMEM((S, 256), u32),
        pltpu.VMEM((S, 512), f32),
        pltpu.VMEM((4, S // 2, 128), u32),
        pltpu.SemaphoreType.DMA((16,)),
    )


def _strassen_a(get, sa_ref, rows):
    a11, a12, a21, a22 = [get(i, j, rows).astype(f32) for i in (0, 1) for j in (0, 1)]
    s1 = a21 + a22
    s2 = s1 - a11
    sa_ref[0, rows, :] = s1.astype(bf16)
    sa_ref[1, rows, :] = s2.astype(bf16)
    sa_ref[2, rows, :] = (a11 - a21).astype(bf16)
    sa_ref[3, rows, :] = (a12 - s2).astype(bf16)


def _project(get_a, sa_ref, wu, tb, out_ref, n_it, kh, k2, scale=None, extra=None, mid=None):
    rc = 256
    nch = (S // 2) // rc

    def prep(it, slot, c0, cn):
        w, hp = it // 8, it % 8

        def rows(base):
            return jnp.concatenate(
                [x[w, pl.ds(hp + 8 * base, cn, stride=8), :] for x in wu], axis=1)
        ua = rows(c0)
        b11, b12 = _lo(ua), _hi(ua)
        if c0 + cn <= k2:
            ub = rows(kh + c0)
            b21, b22 = _lo(ub), _hi(ub)
            t1 = b12 - b11
            t2 = b22 - t1
            ts = [b11, b21, b22, t2 - b21, t1, t2, b22 - b12]
        else:
            assert c0 >= k2
            z = jnp.zeros_like(b11)
            t1 = b12 - b11
            ts = [b11, z, z, -t1, t1, -t1, -b12]
        for i in range(7):
            tb[slot, i, c0:c0 + cn, :] = ts[i].astype(bf16)

    def aop(i, r0):
        r = slice(r0, r0 + rc)
        return [lambda: get_a(0, 0, r), lambda: get_a(0, 1, r), lambda: sa_ref[3, r, :],
                lambda: get_a(1, 1, r), lambda: sa_ref[0, r, :], lambda: sa_ref[1, r, :],
                lambda: sa_ref[2, r, :]][i]()

    def body(extra, it, _):
        slot = it % 2
        w, hp = it // 8, it % 8
        nxt = jnp.minimum(it + 1, n_it - 1)
        cn = kh // nch
        for ci in range(nch):
            r0 = ci * rc
            p1, p2, p3, p4, p5, p6, p7 = [
                jnp.dot(aop(i, r0), tb[slot, i], preferred_element_type=f32) for i in range(7)]
            u2 = p1 + p6
            u3 = u2 + p7
            res = (p1 + p2, (u2 + p5) + p3, u3 - p4, u3 + p5)
            if scale is not None:
                res = [x * np.float32(scale) for x in res]
            for n, x in enumerate(res):
                r = (n // 2) * (S // 2) + r0
                out_ref[w, 2 * hp + n % 2, r:r + rc, :] = x.astype(bf16)
            prep(nxt, 1 - slot, ci * cn, cn)
            if extra is not None:
                extra(it, ci)
        return 0

    for ci in range(nch):
        prep(0, 0, ci * (kh // nch), kh // nch)
    if mid is None:
        lax.fori_loop(0, n_it, functools.partial(body, None), 0)
    else:
        lax.fori_loop(0, n_it // 2, functools.partial(body, None), 0)
        mid()
        lax.fori_loop(n_it // 2, n_it, functools.partial(body, extra), 0)


def _rowred(x, op):
    r = x[:, :128]
    for t in range(1, x.shape[1] // 128):
        r = op(r, x[:, t * 128:(t + 1) * 128])
    return r


def _attention(q_all, k_all, v_all, o_all, s_ref):
    bq = 256
    nq, nt = S // bq, bq // 128
    nslots = s_ref.shape[0]

    def head(h, _):
        q_ref, k_ref, v_ref, o_ref = q_all.at[h], k_all.at[h], v_all.at[h], o_all.at[h]
        slot, free, fresh = {}, [], list(range(nslots))

        def alloc():
            return free.pop() if free else fresh.pop(0)

        def phase_a(i):
            q0 = i * bq
            mx = None
            for k0 in range(0, q0, bq):
                s = lax.dot_general(q_ref[q0:q0 + bq, :], k_ref[k0:k0 + bq, :], NT,
                                    preferred_element_type=f32)
                slot[i, k0] = sl = alloc()
                s_ref[sl] = s
                r = _rowred(s, jnp.maximum)
                mx = r if mx is None else jnp.maximum(mx, r)
            dm = [None] * nt
            slot[i, q0] = sl = alloc()
            for u in range(nt):
                k0 = q0 + u * 128
                s = lax.dot_general(q_ref[k0:q0 + bq, :], k_ref[k0:k0 + 128, :], NT,
                                    preferred_element_type=f32)
                r = lax.broadcasted_iota(jnp.int32, (128, 128), 0)
                c = lax.broadcasted_iota(jnp.int32, (128, 128), 1)
                d = jnp.where(c <= r, s[:128], NEG)
                s_ref[sl, u * 128:(u + 1) * 128, u * 128:(u + 1) * 128] = d
                dm[u] = d if dm[u] is None else jnp.maximum(dm[u], d)
                if u + 1 < nt:
                    s_ref[sl, (u + 1) * 128:, u * 128:(u + 1) * 128] = s[128:]
                    for t in range(u + 1, nt):
                        x = s[(t - u) * 128:(t - u + 1) * 128]
                        dm[t] = x if dm[t] is None else jnp.maximum(dm[t], x)
            dmc = jnp.concatenate(dm, axis=0)
            if mx is not None:
                dmc = jnp.maximum(dmc, mx)
            return jnp.max(dmc, axis=1, keepdims=True)

        def phase_b(i, m):
            q0 = i * bq
            acc = l = None
            for k0 in range(0, q0, bq):
                sl = slot[i, k0]
                p = jnp.exp2(s_ref[sl] - m)
                free.append(sl)
                x = _rowred(p, jnp.add)
                l = x if l is None else l + x
                o = jnp.dot(p.astype(bf16), v_ref[k0:k0 + bq, :], preferred_element_type=f32)
                acc = o if acc is None else acc + o
            accs, ls = [None] * nt, [None] * nt
            sl = slot[i, q0]
            for u in range(nt):
                k0 = q0 + u * 128
                p = jnp.exp2(s_ref[sl, u * 128:, u * 128:(u + 1) * 128] - m[u * 128:])
                o = jnp.dot(p.astype(bf16), v_ref[k0:k0 + 128, :], preferred_element_type=f32)
                for t in range(u, nt):
                    ot = o[(t - u) * 128:(t - u + 1) * 128]
                    lt = p[(t - u) * 128:(t - u + 1) * 128]
                    accs[t] = ot if accs[t] is None else accs[t] + ot
                    ls[t] = lt if ls[t] is None else ls[t] + lt
            free.append(sl)
            for t in range(nt):
                a, lt = accs[t], ls[t]
                if acc is not None:
                    a = a + acc[t * 128:(t + 1) * 128]
                    lt = lt + l[t * 128:(t + 1) * 128]
                lt = jnp.sum(lt, axis=1, keepdims=True)
                o_ref[q0 + t * 128:q0 + (t + 1) * 128, :] = (a * (1.0 / lt)).astype(bf16)

        ms = [None] * nq
        ms[nq - 1] = phase_a(nq - 1)
        for i in range(nq - 1, -1, -1):
            if i > 0:
                ms[i - 1] = phase_a(i - 1)
            phase_b(i, ms[i])
        return 0

    lax.fori_loop(0, H, head, 0)


def _kernel(xa_hbm, wr_hbm, wi_hbm, xb_hbm, ckv_hbm, wq_hbm, wuk_hbm, wuv_hbm, wot_hbm,
            fd_hbm, gf_hbm, gi_hbm, gdt_hbm, out_hbm,
            at, xbt, xb, sx, ckv, wq0, wq1, wk0, wk1, wot, sem):
    def wcopies(w_hbm, d0, d1, s0):
        return [pltpu.make_async_copy(w_hbm.at[:, pl.ds(0, 128)], d0.bitcast(bf16), sem.at[s0]),
                pltpu.make_async_copy(w_hbm.at[:, pl.ds(128, 128)], d1.bitcast(bf16), sem.at[s0 + 1])]
    cp_xb = pltpu.make_async_copy(xb_hbm, xbt, sem.at[0])
    cp_ckv = pltpu.make_async_copy(ckv_hbm, ckv, sem.at[1])
    cp_wq = wcopies(wq_hbm, wq0.at[0], wq1.at[0], 2)
    cp_wk = wcopies(wuk_hbm, wk0.at[0], wk1.at[0], 4)
    cp_wv = wcopies(wuv_hbm, wk0.at[1], wk1.at[1], 6)
    cp_wo = pltpu.make_async_copy(wot_hbm, wot, sem.at[8])
    hs = S // 2

    def start_b():
        cp_xb.start()
        for c in cp_wq:
            c.start()

    def get_x(i, j, r):
        return xb[i * hs + r.start:i * hs + r.stop, j * 256:(j + 1) * 256]

    def get_c(i, j, r):
        if isinstance(r, slice):
            return ckv[i * hs + r.start:i * hs + r.stop, j * 512:(j + 1) * 512]
        return ckv[pl.ds(i * hs + r.start, r.size), j * 512:(j + 1) * 512]

    def late(c):
        if c == 0:
            cp_xb.wait()
            cp_ckv.start()
            xb[:, DM:] = jnp.zeros((S, 512 - DM), bf16)
        if c < 2:
            for i in range(2):
                r = slice(i * hs + c * 512, i * hs + c * 512 + 512)
                xb[r, :DM] = xbt[:, r].T
        else:
            _strassen_a(get_x, sx, slice((c - 2) * 512, (c - 1) * 512))

    with _scope("A"):
        _spectral(xa_hbm, wr_hbm, wi_hbm, fd_hbm, gf_hbm, gi_hbm, gdt_hbm, at, start_b, late)

    def rest(q, kv):
        def proj(sc, tbq, tb):
            with _scope("wait_wq"):
                for c in cp_wq:
                    c.wait()
            for c in cp_wk:
                c.start()

            def mid():
                cp_ckv.wait()
                for c in cp_wv:
                    c.start()
                cp_wo.start()

            def extra(it, ci):
                rows = pl.ds(pl.multiple_of(((it - 4) * 4 + ci) * 64, 64), 64)
                _strassen_a(get_c, sc, rows)

            with _scope("Qproj"):
                _project(get_x, sx, (wq0, wq1), tbq, q, 8, 256, 192,
                         scale=np.log2(np.e) / 16.0, extra=extra, mid=mid)
            for c in cp_wk + cp_wv:
                c.wait()
            with _scope("KVproj"):
                _project(get_c, sc, (wk0, wk1), tb, kv, 16, 512, 512)

        pl.run_scoped(
            proj,
            pltpu.VMEM((4, S // 2, 512), bf16),
            pltpu.VMEM((2, 7, 256, 256), bf16),
            pltpu.VMEM((2, 7, 512, 256), bf16),
        )

        def attn(o, s_ref, outv, osem):
            with _scope("attn"):
                _attention(q.at[0], kv.at[0], kv.at[1], o, s_ref)
            cp_wo.wait()
            qc = 512
            cps = []
            for c in range(S // qc):
                with _scope("out%d" % c):
                    rows = slice(c * qc, (c + 1) * qc)
                    wo = jnp.concatenate([wot[h] for h in range(H)], axis=1)
                    oc = jnp.concatenate([o[h, rows, :] for h in range(H)], axis=1)
                    bt = lax.dot_general(wo, oc, NT, preferred_element_type=f32)
                    outv[rows, :] = jnp.concatenate([at[:, rows], bt.astype(bf16)], axis=0).T
                    cp = pltpu.make_async_copy(outv.at[rows, :], out_hbm.at[rows, :], osem.at[c])
                    cp.start()
                    cps.append(cp)
            with _scope("tail"):
                for cp in cps:
                    cp.wait()

        pl.run_scoped(
            attn,
            pltpu.VMEM((H, S, HD), bf16),
            pltpu.VMEM((15, 256, 256), f32),
            pltpu.VMEM((S, 2 * DM), bf16),
            pltpu.SemaphoreType.DMA((4,)),
        )

    pl.run_scoped(rest, pltpu.VMEM((1, H, S, HD), bf16), pltpu.VMEM((2, H, S, HD), bf16))


@jax.jit
def pallas_concat_heads__spectral_gfnet__compressed_kv_cla__prompt_kernel(
    A_x: jax.Array,
    A_w_r: jax.Array,
    A_w_i: jax.Array,
    B_x: jax.Array,
    B_c_kv: jax.Array,
    B_w_q: jax.Array,
    B_w_uk: jax.Array,
    B_w_uv: jax.Array,
    B_w_o: jax.Array,
):
    hbm = pl.BlockSpec(memory_space=pltpu.HBM)
    out = pl.pallas_call(
        _kernel,
        out_shape=jax.ShapeDtypeStruct((S, 2 * DM), bf16),
        in_specs=[hbm] * 13,
        out_specs=hbm,
        scratch_shapes=[
            pltpu.VMEM((DM, S), bf16),
            pltpu.VMEM((DM, S), bf16),
            pltpu.VMEM((S, 512), bf16),
            pltpu.VMEM((4, S // 2, 256), bf16),
            pltpu.VMEM((S, DC), bf16),
            pltpu.VMEM((1, DM * H // 2, 128), u32),
            pltpu.VMEM((1, DM * H // 2, 128), u32),
            pltpu.VMEM((2, DC * H // 2, 128), u32),
            pltpu.VMEM((2, DC * H // 2, 128), u32),
            pltpu.VMEM((H, DM, HD), bf16),
            pltpu.SemaphoreType.DMA((9,)),
        ],
        compiler_params=pltpu.CompilerParams(vmem_limit_bytes=120 * 2**20),
        name="gfnet_cla",
    )(
        A_x[0].T, A_w_r.T, A_w_i.T, B_x[0].T, B_c_kv[0],
        B_w_q.reshape(DM * H, HD), B_w_uk.reshape(DC * H, HD), B_w_uv.reshape(DC * H, HD),
        B_w_o.transpose(0, 2, 1),
        jnp.asarray(_FD), jnp.asarray(_GF), jnp.asarray(_GI), jnp.asarray(_GDT),
    )
    return out.reshape(1, S, 2 * DM)
```

```python
import contextlib
import functools

import jax
import jax.numpy as jnp
import ml_dtypes
import numpy as np
from jax import lax
import jax.experimental.pallas as pl
import jax.experimental.pallas.tpu as pltpu

bf16 = jnp.bfloat16
f32 = jnp.float32
u32 = jnp.uint32

S = 2048
DM = 448
F = 225
N1, N2 = 16, 128
H, HD = 16, 256
DC = 1024
NT = (((1,), (1,)), ((), ()))
NEG = -1e30
_OUT_UNROLL = [2]
_SCOPES = [False]


def _scope(name):
    return jax.named_scope(name) if _SCOPES[0] else contextlib.nullcontext()


def _dft_constants():
    d = np.arange(DM)[:, None]
    f = np.arange(F)[None, :]
    th = 2 * np.pi * ((d * f) % DM) / DM
    fd = np.zeros((DM, 512))
    fd[:, :F] = np.cos(th)
    fd[:, 256:256 + F] = -np.sin(th)
    k1 = np.arange(N1)[:, None, None]
    k2 = np.arange(N2)[None, :, None]
    n2 = np.arange(N2)[None, None, :]
    ang = 2 * np.pi * ((n2 * (k1 + N1 * k2)) % S) / S
    gr, gi_ = np.cos(ang), -np.sin(ang)
    gf = np.zeros((N1, 256, 256))
    gf[:, :128, 0::2] = gr
    gf[:, :128, 1::2] = -gi_
    gf[:, 128:, 0::2] = gi_
    gf[:, 128:, 1::2] = gr
    grt, git = gr.transpose(0, 2, 1), gi_.transpose(0, 2, 1)
    gi = np.zeros((N1, 256, 256))
    gi[:, :128, 0::2] = grt
    gi[:, :128, 1::2] = git
    gi[:, 128:, 0::2] = -git
    gi[:, 128:, 1::2] = grt
    c = np.full(F, 2.0)
    c[0] = 1
    c[-1] = 1
    gdt = np.zeros((DM, 512))
    gdt[:, :F] = c[None, :] * np.cos(th) / (S * DM)
    gdt[:, 256:256 + F] = -c[None, :] * np.sin(th) / (S * DM)
    cv = lambda a: a.astype(np.float32).astype(ml_dtypes.bfloat16)
    return cv(fd), cv(gf), cv(gi), cv(gdt)


_FD, _GF, _GI, _GDT = _dft_constants()


class _SV:
    __slots__ = ("v", "s")

    def __init__(self, v, s=1):
        self.v = v
        self.s = s

    def __neg__(self):
        return _SV(self.v, -self.s)

    def __add__(self, b):
        if self.s > 0 and b.s > 0:
            return _SV(self.v + b.v)
        if self.s > 0:
            return _SV(self.v - b.v)
        if b.s > 0:
            return _SV(b.v - self.v)
        return _SV(self.v + b.v, -1)

    def __sub__(self, b):
        return self + (-b)

    def scale(self, c):
        return _SV(self.v * np.float32(abs(c)), self.s * (1 if c > 0 else -1))

    def get(self):
        return self.v if self.s > 0 else -self.v


def _twiddle(x, j, n, sign):
    re, im = x
    j %= n
    if j == 0:
        return x
    if 4 * j == n:
        return (im, -re) if sign < 0 else (-im, re)
    if 2 * j == n:
        return (-re, -im)
    if 4 * j == 3 * n:
        return (-im, re) if sign < 0 else (im, -re)
    c = np.cos(2 * np.pi * j / n)
    s = sign * np.sin(2 * np.pi * j / n)
    if (8 * j) % n == 0:
        h = np.sqrt(0.5)
        r = (re if c > 0 else -re) - (im if s > 0 else -im)
        i = (im if c > 0 else -im) + (re if s > 0 else -re)
        return (r.scale(h), i.scale(h))
    return (re.scale(c) - im.scale(s), im.scale(c) + re.scale(s))


def _fft(xs, sign):
    n = len(xs)
    if n == 1:
        return xs
    h = n // 2
    ev = [(xs[j][0] + xs[j + h][0], xs[j][1] + xs[j + h][1]) for j in range(h)]
    od = [_twiddle((xs[j][0] - xs[j + h][0], xs[j][1] - xs[j + h][1]), j, n, sign)
          for j in range(h)]
    out = [None] * n
    out[0::2] = _fft(ev, sign)
    out[1::2] = _fft(od, sign)
    return out


def _lo(u):
    return pltpu.bitcast(u << 16, f32)


def _hi(u):
    return pltpu.bitcast(u & np.uint32(0xFFFF0000), f32)


def _spectral(xa_hbm, wr_hbm, wi_hbm, fd_hbm, gf_hbm, gi_hbm, gdt_hbm, at_ref, start_b, late):
    def body(xa, wraw, fd, gf, gi, gdt, x1, upk, vv, wu, sem):
        cp_fd = pltpu.make_async_copy(fd_hbm, fd, sem.at[0])
        cp_xa = [pltpu.make_async_copy(xa_hbm.at[:, pl.ds(c * 512, 512)],
                                       xa.at[:, pl.ds(c * 512, 512)], sem.at[1 + c])
                 for c in range(4)]
        cp_wr = pltpu.make_async_copy(wr_hbm, wraw.at[0], sem.at[5])
        cp_wi = pltpu.make_async_copy(wi_hbm, wraw.at[1], sem.at[6])
        cp_gd = pltpu.make_async_copy(gdt_hbm, gdt, sem.at[7])
        cp_g = [[pltpu.make_async_copy(h.at[pl.ds(4 * j, 4)], v.at[pl.ds(4 * j, 4)],
                                       sem.at[8 + 2 * j + n])
                 for n, (h, v) in enumerate(((gf_hbm, gf), (gi_hbm, gi)))] for j in range(4)]
        cp_fd.start()
        for c in cp_xa:
            c.start()
        with _scope("A0wait"):
            cp_fd.wait()
            cp_xa[0].wait()
        for c in range(4):
            with _scope("A1_%d" % c):
                if c:
                    cp_xa[c].wait()
                if c == 0:
                    for cp in (cp_wr, cp_wi):
                        cp.start()
                if c == 1:
                    for cp in cp_g[0]:
                        cp.start()
                if c == 2:
                    for cp in cp_g[1]:
                        cp.start()
                xs = xa[:, c * 512:(c + 1) * 512].T
                x1[c * 512:(c + 1) * 512, :] = jnp.dot(xs, fd[...], preferred_element_type=f32)
        with _scope("A2"):
            for r8 in range(16):
                for t in range(2):
                    rows = lambda n: slice(128 * n + 8 * r8, 128 * n + 8 * r8 + 8)
                    xs = [(_SV(x1[rows(n), 128 * t:128 * t + 128]),
                           _SV(x1[rows(n), 256 + 128 * t:256 + 128 * t + 128])) for n in range(16)]
                    ys = _fft(xs, -1)
                    for k in range(16):
                        upk[rows(k), 128 * t:128 * t + 128] = pltpu.pack_elementwise(
                            [ys[k][0].get(), ys[k][1].get()], packed_dtype=bf16)
            cp_wr.wait()
            cp_wi.wait()
            for cp in cp_g[2] + cp_g[3] + [cp_gd]:
                cp.start()
            for a in range(2):
                w = jnp.concatenate([wraw[a], jnp.zeros((256 - F, S), bf16)], axis=0).T
                w = pltpu.bitcast(w, u32)
                wu[a * 2] = w[:, :128]
                wu[a * 2 + 1] = w[:, 128:]
        with _scope("A3"):
            for j in range(8):
                if j % 4 == 0:
                    for cp in cp_g[j // 2] + cp_g[j // 2 + 1]:
                        cp.wait()
                if j == 4:
                    start_b()
                wq = [jnp.concatenate([wu[a * 2 + t, pl.ds(j, 128, stride=8), :]
                                       for t in range(2)], axis=1) for a in range(2)]
                for b in range(2):
                    k1 = 2 * j + b
                    y = jnp.dot(gf[k1], pltpu.bitcast(upk[128 * k1:128 * k1 + 128, :], bf16),
                                preferred_element_type=f32)
                    yr, yi = y[:128], y[128:]
                    wr, wi = [(_lo if b == 0 else _hi)(w) for w in wq]
                    zr = yr * wr - yi * wi
                    zi = yr * wi + yi * wr
                    zp = pltpu.bitcast(pltpu.pack_elementwise([zr, zi], packed_dtype=bf16), bf16)
                    v = jnp.dot(gi[k1], zp, preferred_element_type=f32)
                    vv[128 * k1:128 * k1 + 128, 0:256] = v[:128]
                    vv[128 * k1:128 * k1 + 128, 256:512] = v[128:]
        with _scope("A6"):
            for r8 in range(16):
                for t in range(2):
                    rows = lambda n: slice(128 * n + 8 * r8, 128 * n + 8 * r8 + 8)
                    xs = [(_SV(vv[rows(n), 128 * t:128 * t + 128]),
                           _SV(vv[rows(n), 256 + 128 * t:256 + 128 * t + 128])) for n in range(16)]
                    ys = _fft(xs, +1)
                    for k in range(16):
                        x1[rows(k), 128 * t:128 * t + 128] = ys[k][0].get()
                        x1[rows(k), 256 + 128 * t:256 + 128 * t + 128] = ys[k][1].get()
        with _scope("A7"):
            cp_gd.wait()
            for c in range(4):
                tt = x1[c * 512:(c + 1) * 512, :].astype(bf16)
                at_ref[:, c * 512:(c + 1) * 512] = lax.dot_general(
                    gdt[...], tt, NT, preferred_element_type=f32).astype(bf16)
                late(c)

    pl.run_scoped(
        body,
        pltpu.VMEM((DM, S), bf16),
        pltpu.VMEM((2, F, S), bf16),
        pltpu.VMEM((DM, 512), bf16),
        pltpu.VMEM((N1, 256, 256), bf16),
        pltpu.VMEM((N1, 256, 256), bf16),
        pltpu.VMEM((DM, 512), bf16),
        pltpu.VMEM((S, 512), f32),
        pltpu.VMEM((S, 256), u32),
        pltpu.VMEM((S, 512), f32),
        pltpu.VMEM((4, S // 2, 128), u32),
        pltpu.SemaphoreType.DMA((16,)),
    )


def _strassen_a(get, sa_ref, rows):
    a11, a12, a21, a22 = [get(i, j, rows).astype(f32) for i in (0, 1) for j in (0, 1)]
    s1 = a21 + a22
    s2 = s1 - a11
    sa_ref[0, rows, :] = s1.astype(bf16)
    sa_ref[1, rows, :] = s2.astype(bf16)
    sa_ref[2, rows, :] = (a11 - a21).astype(bf16)
    sa_ref[3, rows, :] = (a12 - s2).astype(bf16)


def _project(get_a, sa_ref, wu, tb, out_ref, n_it, kh, k2, scale=None, extra=None, mid=None):
    rc = 256
    nch = (S // 2) // rc

    def prep(it, slot, c0, cn):
        w, hp = it // 8, it % 8

        def rows(base):
            return jnp.concatenate(
                [x[w, pl.ds(hp + 8 * base, cn, stride=8), :] for x in wu], axis=1)
        ua = rows(c0)
        b11, b12 = _lo(ua), _hi(ua)
        if c0 + cn <= k2:
            ub = rows(kh + c0)
            b21, b22 = _lo(ub), _hi(ub)
            t1 = b12 - b11
            t2 = b22 - t1
            ts = [b11, b21, b22, t2 - b21, t1, t2, b22 - b12]
        else:
            assert c0 >= k2
            z = jnp.zeros_like(b11)
            t1 = b12 - b11
            ts = [b11, z, z, -t1, t1, -t1, -b12]
        for i in range(7):
            tb[slot, i, c0:c0 + cn, :] = ts[i].astype(bf16)

    def aop(i, r0):
        r = slice(r0, r0 + rc)
        return [lambda: get_a(0, 0, r), lambda: get_a(0, 1, r), lambda: sa_ref[3, r, :],
                lambda: get_a(1, 1, r), lambda: sa_ref[0, r, :], lambda: sa_ref[1, r, :],
                lambda: sa_ref[2, r, :]][i]()

    def body(extra, it, _):
        slot = it % 2
        w, hp = it // 8, it % 8
        nxt = jnp.minimum(it + 1, n_it - 1)
        cn = kh // nch
        for ci in range(nch):
            r0 = ci * rc
            p1, p2, p3, p4, p5, p6, p7 = [
                jnp.dot(aop(i, r0), tb[slot, i], preferred_element_type=f32) for i in range(7)]
            u2 = p1 + p6
            u3 = u2 + p7
            res = (p1 + p2, (u2 + p5) + p3, u3 - p4, u3 + p5)
            if scale is not None:
                res = [x * np.float32(scale) for x in res]
            for n, x in enumerate(res):
                r = (n // 2) * (S // 2) + r0
                out_ref[w, 2 * hp + n % 2, r:r + rc, :] = x.astype(bf16)
            prep(nxt, 1 - slot, ci * cn, cn)
            if extra is not None:
                extra(it, ci)
        return 0

    for ci in range(nch):
        prep(0, 0, ci * (kh // nch), kh // nch)
    if mid is None:
        lax.fori_loop(0, n_it, functools.partial(body, None), 0)
    else:
        lax.fori_loop(0, n_it // 2, functools.partial(body, None), 0)
        mid()
        lax.fori_loop(n_it // 2, n_it, functools.partial(body, extra), 0)


def _s_a(a):
    return [a[0] + a[3], a[2] + a[3], a[0], a[3], a[0] + a[1], a[2] - a[0], a[1] - a[3]]


def _s_b(b):
    return [b[0] + b[3], b[0], b[1] - b[3], b[2] - b[0], b[3], b[0] + b[1], b[2] + b[3]]


def _s_c(m):
    return [m[0] + m[3] - m[4] + m[6], m[2] + m[4], m[1] + m[3], m[0] - m[1] + m[2] + m[5]]


_PLAIN = {2: 0, 3: 3}
_AIDX = {}
for _so in range(7):
    for _si in range(7):
        if not (_so in _PLAIN and _si in _PLAIN):
            _AIDX[_so, _si] = len(_AIDX)


def _kv_ablk(ckv, io, ii, r):
    mo, ko = divmod(io, 2)
    mi, ki = divmod(ii, 2)
    c0 = ko * 512 + ki * 256
    if isinstance(r, slice):
        rows = slice(mo * 1024 + mi * 512 + r.start, mo * 1024 + mi * 512 + r.stop)
    else:
        rows = pl.ds(mo * 1024 + mi * 512 + r.start, r.size)
    return ckv[rows, c0:c0 + 256]


def _kv_sums(ckv, sc, r):
    out = [_s_a([_kv_ablk(ckv, io, ii, r).astype(f32) for io in range(4)]) for ii in range(4)]
    for so in range(7):
        ops = _s_a([out[ii][so] for ii in range(4)])
        for si in range(7):
            if (so, si) in _AIDX:
                sc[_AIDX[so, si], r, :] = ops[si].astype(bf16)


def _kv_project(ckv, sc, wu, tb, kv):
    rc = 256
    nch = 512 // rc

    def prep(hp, slot, c0, cn):
        u = {}
        for no in range(2):
            for kk in range(4):
                u[no, kk] = jnp.concatenate(
                    [x[no, pl.ds(hp + 8 * (kk * 256 + c0), cn, stride=8), :] for x in wu], axis=1)
        out = [_s_b([(_lo if ji % 2 == 0 else _hi)(u[jo % 2, 2 * (jo // 2) + ji // 2])
                     for jo in range(4)]) for ji in range(4)]
        for so in range(7):
            ops = _s_b([out[ji][so] for ji in range(4)])
            for si in range(7):
                tb[slot, so * 7 + si, c0:c0 + cn, :] = ops[si].astype(bf16)

    def aop(so, si, r):
        if (so, si) in _AIDX:
            return sc[_AIDX[so, si], r, :]
        return _kv_ablk(ckv, _PLAIN[so], _PLAIN[si], r)

    def body(hp, _):
        slot = hp % 2
        nxt = jnp.minimum(hp + 1, H // 2 - 1)
        k = 0
        for ci in range(nch):
            r = slice(ci * rc, ci * rc + rc)
            d = []
            for so in range(7):
                m = [jnp.dot(aop(so, si, r), tb[slot, so * 7 + si], preferred_element_type=f32)
                     for si in range(7)]
                d.append(_s_c(m))
                a = (k * 16 // (nch * 7)) * 16
                b = ((k + 1) * 16 // (nch * 7)) * 16
                k += 1
                if b > a:
                    prep(nxt, 1 - slot, a, b - a)
            for cin in range(4):
                c = _s_c([d[so][cin] for so in range(7)])
                mi, ni = divmod(cin, 2)
                for co in range(4):
                    mo, no = divmod(co, 2)
                    r0 = mo * 1024 + mi * 512
                    kv[no, 2 * hp + ni, r0 + r.start:r0 + r.stop, :] = c[co].astype(bf16)
        return 0

    for c0 in range(0, 256, 64):
        prep(0, 0, c0, 64)
    lax.fori_loop(0, H // 2, body, 0)


def _rowred(x, op):
    r = x[:, :128]
    for t in range(1, x.shape[1] // 128):
        r = op(r, x[:, t * 128:(t + 1) * 128])
    return r


def _attention(q_all, k_all, v_all, o_all, s_ref):
    bq = 256
    nq, nt = S // bq, bq // 128
    nslots = s_ref.shape[0]

    def head(h, _):
        q_ref, k_ref, v_ref, o_ref = q_all.at[h], k_all.at[h], v_all.at[h], o_all.at[h]
        slot, free, fresh = {}, [], list(range(nslots))

        def alloc():
            return free.pop() if free else fresh.pop(0)

        def phase_a(i):
            q0 = i * bq
            mx = None
            for k0 in range(0, q0, bq):
                s = lax.dot_general(q_ref[q0:q0 + bq, :], k_ref[k0:k0 + bq, :], NT,
                                    preferred_element_type=f32)
                slot[i, k0] = sl = alloc()
                s_ref[sl] = s
                r = _rowred(s, jnp.maximum)
                mx = r if mx is None else jnp.maximum(mx, r)
            dm = [None] * nt
            slot[i, q0] = sl = alloc()
            for u in range(nt):
                k0 = q0 + u * 128
                s = lax.dot_general(q_ref[k0:q0 + bq, :], k_ref[k0:k0 + 128, :], NT,
                                    preferred_element_type=f32)
                r = lax.broadcasted_iota(jnp.int32, (128, 128), 0)
                c = lax.broadcasted_iota(jnp.int32, (128, 128), 1)
                d = jnp.where(c <= r, s[:128], NEG)
                s_ref[sl, u * 128:(u + 1) * 128, u * 128:(u + 1) * 128] = d
                dm[u] = d if dm[u] is None else jnp.maximum(dm[u], d)
                if u + 1 < nt:
                    s_ref[sl, (u + 1) * 128:, u * 128:(u + 1) * 128] = s[128:]
                    for t in range(u + 1, nt):
                        x = s[(t - u) * 128:(t - u + 1) * 128]
                        dm[t] = x if dm[t] is None else jnp.maximum(dm[t], x)
            dmc = jnp.concatenate(dm, axis=0)
            if mx is not None:
                dmc = jnp.maximum(dmc, mx)
            return jnp.max(dmc, axis=1, keepdims=True)

        def phase_b(i, m):
            q0 = i * bq
            acc = l = None
            for k0 in range(0, q0, bq):
                sl = slot[i, k0]
                p = jnp.exp2(s_ref[sl] - m)
                free.append(sl)
                x = _rowred(p, jnp.add)
                l = x if l is None else l + x
                o = jnp.dot(p.astype(bf16), v_ref[k0:k0 + bq, :], preferred_element_type=f32)
                acc = o if acc is None else acc + o
            accs, ls = [None] * nt, [None] * nt
            sl = slot[i, q0]
            for u in range(nt):
                k0 = q0 + u * 128
                p = jnp.exp2(s_ref[sl, u * 128:, u * 128:(u + 1) * 128] - m[u * 128:])
                o = jnp.dot(p.astype(bf16), v_ref[k0:k0 + 128, :], preferred_element_type=f32)
                for t in range(u, nt):
                    ot = o[(t - u) * 128:(t - u + 1) * 128]
                    lt = p[(t - u) * 128:(t - u + 1) * 128]
                    accs[t] = ot if accs[t] is None else accs[t] + ot
                    ls[t] = lt if ls[t] is None else ls[t] + lt
            free.append(sl)
            for t in range(nt):
                a, lt = accs[t], ls[t]
                if acc is not None:
                    a = a + acc[t * 128:(t + 1) * 128]
                    lt = lt + l[t * 128:(t + 1) * 128]
                lt = jnp.sum(lt, axis=1, keepdims=True)
                o_ref[q0 + t * 128:q0 + (t + 1) * 128, :] = (a * (1.0 / lt)).astype(bf16)

        ms = [None] * nq
        ms[nq - 1] = phase_a(nq - 1)
        for i in range(nq - 1, -1, -1):
            if i > 0:
                ms[i - 1] = phase_a(i - 1)
            phase_b(i, ms[i])
        return 0

    lax.fori_loop(0, H, head, 0)


def _kernel(xa_hbm, wr_hbm, wi_hbm, xb_hbm, ckv_hbm, wq_hbm, wuk_hbm, wuv_hbm, wot_hbm,
            fd_hbm, gf_hbm, gi_hbm, gdt_hbm, out_hbm,
            at, xbt, xb, sx, ckv, wq0, wq1, wk0, wk1, wot, sem):
    def wcopies(w_hbm, d0, d1, s0):
        return [pltpu.make_async_copy(w_hbm.at[:, pl.ds(0, 128)], d0.bitcast(bf16), sem.at[s0]),
                pltpu.make_async_copy(w_hbm.at[:, pl.ds(128, 128)], d1.bitcast(bf16), sem.at[s0 + 1])]
    cp_xb = pltpu.make_async_copy(xb_hbm, xbt, sem.at[0])
    cp_ckv = pltpu.make_async_copy(ckv_hbm, ckv, sem.at[1])
    cp_wq = wcopies(wq_hbm, wq0.at[0], wq1.at[0], 2)
    cp_wk = wcopies(wuk_hbm, wk0.at[0], wk1.at[0], 4)
    cp_wv = wcopies(wuv_hbm, wk0.at[1], wk1.at[1], 6)
    cp_wo = pltpu.make_async_copy(wot_hbm, wot, sem.at[8])
    hs = S // 2

    def start_b():
        cp_xb.start()
        for c in cp_wq:
            c.start()

    def get_x(i, j, r):
        return xb[i * hs + r.start:i * hs + r.stop, j * 256:(j + 1) * 256]

    def get_c(i, j, r):
        if isinstance(r, slice):
            return ckv[i * hs + r.start:i * hs + r.stop, j * 512:(j + 1) * 512]
        return ckv[pl.ds(i * hs + r.start, r.size), j * 512:(j + 1) * 512]

    def late(c):
        if c == 0:
            cp_xb.wait()
            cp_ckv.start()
            xb[:, DM:] = jnp.zeros((S, 512 - DM), bf16)
        if c < 2:
            for i in range(2):
                r = slice(i * hs + c * 512, i * hs + c * 512 + 512)
                xb[r, :DM] = xbt[:, r].T
        else:
            _strassen_a(get_x, sx, slice((c - 2) * 512, (c - 1) * 512))

    with _scope("A"):
        _spectral(xa_hbm, wr_hbm, wi_hbm, fd_hbm, gf_hbm, gi_hbm, gdt_hbm, at, start_b, late)

    def rest(q, kv):
        def proj(sc, tbq, tb):
            with _scope("wait_wq"):
                for c in cp_wq:
                    c.wait()
            for c in cp_wk:
                c.start()

            def mid():
                cp_ckv.wait()
                for c in cp_wv:
                    c.start()
                cp_wo.start()

            def extra(it, ci):
                rows = pl.ds(pl.multiple_of(((it - 4) * 4 + ci) * 32, 32), 32)
                _kv_sums(ckv, sc, rows)

            with _scope("Qproj"):
                _project(get_x, sx, (wq0, wq1), tbq, q, 8, 256, 192,
                         scale=np.log2(np.e) / 16.0, extra=extra, mid=mid)
            for c in cp_wk + cp_wv:
                c.wait()
            with _scope("KVproj"):
                _kv_project(ckv, sc, (wk0, wk1), tb, kv)

        pl.run_scoped(
            proj,
            pltpu.VMEM((len(_AIDX), 512, 256), bf16),
            pltpu.VMEM((2, 7, 256, 256), bf16),
            pltpu.VMEM((2, 49, 256, 256), bf16),
        )

        def attn(o, s_ref, outv, osem):
            with _scope("attn"):
                _attention(q.at[0], kv.at[0], kv.at[1], o, s_ref)
            cp_wo.wait()
            qc = 512

            def out_copy(c):
                rows = pl.ds(pl.multiple_of(c * qc, qc), qc)
                return pltpu.make_async_copy(outv.at[rows, :], out_hbm.at[rows, :], osem.at[c])

            def out_chunk(c, _):
                rows = pl.ds(pl.multiple_of(c * qc, qc), qc)
                wo = jnp.concatenate([wot[h] for h in range(H)], axis=1)
                oc = jnp.concatenate([o[h, rows, :] for h in range(H)], axis=1)
                bt = lax.dot_general(wo, oc, NT, preferred_element_type=f32)
                outv[rows, :] = jnp.concatenate([at[:, rows], bt.astype(bf16)], axis=0).T
                out_copy(c).start()
                return 0

            with _scope("out"):
                lax.fori_loop(0, S // qc, out_chunk, 0, unroll=_OUT_UNROLL[0])
            with _scope("tail"):
                for c in range(S // qc):
                    out_copy(c).wait()

        pl.run_scoped(
            attn,
            pltpu.VMEM((H, S, HD), bf16),
            pltpu.VMEM((15, 256, 256), f32),
            pltpu.VMEM((S, 2 * DM), bf16),
            pltpu.SemaphoreType.DMA((4,)),
        )

    pl.run_scoped(rest, pltpu.VMEM((1, H, S, HD), bf16), pltpu.VMEM((2, H, S, HD), bf16))


@jax.jit
def pallas_concat_heads__spectral_gfnet__compressed_kv_cla__prompt_kernel(
    A_x: jax.Array,
    A_w_r: jax.Array,
    A_w_i: jax.Array,
    B_x: jax.Array,
    B_c_kv: jax.Array,
    B_w_q: jax.Array,
    B_w_uk: jax.Array,
    B_w_uv: jax.Array,
    B_w_o: jax.Array,
):
    hbm = pl.BlockSpec(memory_space=pltpu.HBM)
    out = pl.pallas_call(
        _kernel,
        out_shape=jax.ShapeDtypeStruct((S, 2 * DM), bf16),
        in_specs=[hbm] * 13,
        out_specs=hbm,
        scratch_shapes=[
            pltpu.VMEM((DM, S), bf16),
            pltpu.VMEM((DM, S), bf16),
            pltpu.VMEM((S, 512), bf16),
            pltpu.VMEM((4, S // 2, 256), bf16),
            pltpu.VMEM((S, DC), bf16),
            pltpu.VMEM((1, DM * H // 2, 128), u32),
            pltpu.VMEM((1, DM * H // 2, 128), u32),
            pltpu.VMEM((2, DC * H // 2, 128), u32),
            pltpu.VMEM((2, DC * H // 2, 128), u32),
            pltpu.VMEM((H, DM, HD), bf16),
            pltpu.SemaphoreType.DMA((9,)),
        ],
        compiler_params=pltpu.CompilerParams(vmem_limit_bytes=120 * 2**20),
        name="gfnet_cla",
    )(
        A_x[0].T, A_w_r.T, A_w_i.T, B_x[0].T, B_c_kv[0],
        B_w_q.reshape(DM * H, HD), B_w_uk.reshape(DC * H, HD), B_w_uv.reshape(DC * H, HD),
        B_w_o.transpose(0, 2, 1),
        jnp.asarray(_FD), jnp.asarray(_GF), jnp.asarray(_GI), jnp.asarray(_GDT),
    )
    return out.reshape(1, S, 2 * DM)
```
